```python
import os as _os
_os.environ.setdefault("JAX_PLATFORMS", "cpu")
import jax
import jax.numpy as jnp

def _softmax(x, axis=-1):
    return jax.nn.softmax(x, axis=axis)
def _gelu(x):
    return jax.nn.gelu(x, approximate=True)
def _silu(x):
    return jax.nn.silu(x)
def _sigmoid(x):
    return jax.nn.sigmoid(x)
def _layernorm(x, axis=-1, eps=1e-5):
    m = jnp.mean(x, axis=axis, keepdims=True)
    v = jnp.var(x, axis=axis, keepdims=True)
    return (x - m) / jnp.sqrt(v + eps)
def _scatter_add(tgt, idx, src, axis=0):
    return tgt.at[idx].add(src)
def _segment_sum(src, seg, n):
    return jax.ops.segment_sum(src, seg, n)
class _Rng:
    def __init__(self, key):
        self._k = key
    def _next(self):
        self._k, sub = jax.random.split(self._k)
        return sub
    def normal(self, shape):
        return jax.random.normal(self._next(), shape, dtype=jnp.bfloat16)
    def randint(self, lo, hi, shape):
        return jax.random.randint(self._next(), shape, lo, hi, dtype=jnp.int32)
    def uniform(self, shape, lo=0.0, hi=1.0):
        return jax.random.uniform(self._next(), shape, jnp.bfloat16, lo, hi)
    def permutation(self, n):
        return jax.random.permutation(self._next(), n)


kernel_name = 'standalone__mha_softmax__near_ridge'

def setup_inputs():
    _rng = _Rng(jax.random.key(int.from_bytes(__import__("os").urandom(4), "little")))
    _w = (lambda a: (lambda t: t.astype(jnp.bfloat16) if jnp.issubdtype(t.dtype, jnp.floating) else t)(jnp.asarray(a)))
    B, H, Sq, Sk, D = 8, 32, 496, 512, 192
    return {
        "q": _w((lambda *s: _rng.normal(s) * 0.05)(B, H, Sq, D)),
        "k": _w((lambda *s: _rng.normal(s) * 3.2)(B, H, Sk, D)),
        "v": _w((lambda *s: _rng.normal(s) * 0.05)(B, H, Sk, D)),
    }

def reference(q, k, v):
    scale = q.shape[-1] ** -0.5
    scores = jnp.einsum("bhqd,bhkd->bhqk", q, k) * scale
    p = _softmax(scores, axis=-1)
    return jnp.einsum("bhqk,bhkd->bhqd", p, v)
```

```python
import functools

import jax
import jax.numpy as jnp
from jax import lax
import jax.experimental.pallas as pl
import jax.experimental.pallas.tpu as pltpu

_LOG2E = 1.4426950408889634
_HEADS_PER_STEP = 8


def _mha_kernel(q_ref, k_ref, v_ref, o_ref, *, c, hb):
    def qk(h):
        return lax.dot_general(k_ref[h], q_ref[h], (((0,), (0,)), ((), ())),
                               preferred_element_type=jnp.float32)

    def softmax_pv(h, sT):
        m = jnp.max(sT, axis=0, keepdims=True)
        p = jnp.exp2(sT * c - m * c)
        l = jnp.sum(p, axis=0, keepdims=True)
        oT = jnp.dot(v_ref[h], p.astype(jnp.bfloat16), preferred_element_type=jnp.float32)
        o_ref[h] = (oT * (1.0 / l)).astype(o_ref.dtype)

    s = qk(0)
    for h in range(hb):
        s_next = qk(h + 1) if h + 1 < hb else None
        softmax_pv(h, s)
        s = s_next


@jax.jit
def pallas_standalone__mha_softmax__near_ridge_kernel(
    q: jax.Array,
    k: jax.Array,
    v: jax.Array,
):
    B, H, Sq, D = q.shape
    Sk = k.shape[2]
    hb = _HEADS_PER_STEP
    c = (D ** -0.5) * _LOG2E
    qT = jnp.swapaxes(q, -1, -2).reshape(B * H, D, Sq)
    kT = jnp.swapaxes(k, -1, -2).reshape(B * H, D, Sk)
    vT = jnp.swapaxes(v, -1, -2).reshape(B * H, D, Sk)
    oT = pl.pallas_call(
        functools.partial(_mha_kernel, c=c, hb=hb),
        grid=(B * H // hb,),
        in_specs=[
            pl.BlockSpec((hb, D, Sq), lambda i: (i, 0, 0)),
            pl.BlockSpec((hb, D, Sk), lambda i: (i, 0, 0)),
            pl.BlockSpec((hb, D, Sk), lambda i: (i, 0, 0)),
        ],
        out_specs=pl.BlockSpec((hb, D, Sq), lambda i: (i, 0, 0)),
        out_shape=jax.ShapeDtypeStruct((B * H, D, Sq), q.dtype),
        compiler_params=pltpu.CompilerParams(
            dimension_semantics=("parallel",),
            vmem_limit_bytes=100 * 1024 * 1024,
            flags={"XLA_TPU_FORCE_LP_LLO_SCHEDULER": True},
        ),
    )(qT, kT, vT)
    return jnp.swapaxes(oT.reshape(B, H, D, Sq), -1, -2)
```

```python
import functools

import jax
import jax.numpy as jnp
from jax import lax
import jax.experimental.pallas as pl
import jax.experimental.pallas.tpu as pltpu

_LOG2E = 1.4426950408889634
_G = 18
_R = 6
_g = 2


def _mha_kernel(q_hbm, k_hbm, v_hbm, o_hbm, qb, kb, vb, ob, s_scr, p_scr, r_scr,
                sq, sk, sv, so, *, c, NH):
    G, R, g = _G, _R, _g
    NG = R // g
    ob[R, 0:16, 0:128] = jnp.zeros((16, 128), ob.dtype)
    zz = pl.program_id(0) // 4096

    def cq(h, p, n=g, off=0):
        return pltpu.make_async_copy(q_hbm.at[pl.ds(h, n)], qb.at[pl.ds(p * g + off, n)], sq.at[p])

    def ck(h, p, n=g, off=0):
        return pltpu.make_async_copy(k_hbm.at[pl.ds(h, n)], kb.at[pl.ds(p * g + off, n)], sk.at[p])

    def cv(h, p):
        return pltpu.make_async_copy(v_hbm.at[pl.ds(h, g)], vb.at[pl.ds(p * g, g)], sv.at[p])

    def co(h, p):
        return pltpu.make_async_copy(ob.at[pl.ds(p * g, g)], o_hbm.at[pl.ds(h, g)], so.at[p])

    def when(cond, fn):
        if isinstance(cond, bool):
            if cond:
                fn()
        else:
            pl.when(cond)(fn)

    def lanes(x, op):
        parts = [x[:, i * 128:(i + 1) * 128] for i in range(x.shape[1] // 128)]
        while len(parts) > 1:
            parts = [op(parts[2 * i], parts[2 * i + 1]) for i in range(len(parts) // 2)]
        return parts[0]

    def qk(slot, ss):
        s_scr[ss] = lax.dot_general(qb[slot], kb[slot], (((0,), (0,)), ((), ())),
                                    preferred_element_type=jnp.float32)

    def sm(ss):
        s = s_scr[ss]
        m = jnp.max(lanes(s, jnp.maximum), axis=1, keepdims=True)
        p = jnp.exp2((s - m) * c)
        pb = p.astype(jnp.bfloat16)
        ps = lanes(pb.astype(jnp.float32), jnp.add)
        r = 1.0 / jnp.sum(ps, axis=1, keepdims=True).T
        return pb, r

    def pv(slot, pr):
        pb, r = pr
        oT = lax.dot_general(vb[slot], pb, (((1,), (1,)), ((), ())),
                             preferred_element_type=jnp.float32)
        return oT, r

    def fin(slot, orr):
        oT, r = orr
        ob[slot] = (oT * r).astype(ob.dtype)
        qb[R + zz, 0:16, 0:128] = ob[R + zz, 0:16, 0:128]

    def finish(u, slot, pend):
        p = slot // g
        if slot % g == 0:
            when(u >= R, lambda: co(u - R, p).wait())
        fin(slot, pend)
        if slot % g == g - 1:
            co(u + 1 - g, p).start()

    def step(u0, j, st, do_qk=True, do_sm=True, last=False):
        pr, pend = st
        u = u0 + j
        slot = j % R
        p = slot // g
        if do_qk:
            if slot % g == 0:
                cq(u + 2, p).wait()
                ck(u + 2, p).wait()
            qk(slot, j % 2)
            if slot % g == g - 1:
                hq = u + 1 - g + R + 2

                def _():
                    cq(hq, p).start()
                    ck(hq, p).start()
                when(hq + g <= NH, _)
        if pend is not None:
            finish(u - 1, (j - 1) % R, pend)
        prn = sm((j + 1) % 2) if do_sm else None
        if slot % g == 0:
            cv(u, p).wait()
        pend = pv(slot, pr)
        if slot % g == g - 1:
            hv = u + 1 - g + R
            when(hv + g <= NH, lambda: cv(hv, p).start())
        if last:
            finish(u, slot, pend)
            pend = None
        return prn, pend

    def set_a(p):
        if p < NG - 1:
            cq(2 + p * g, p).start()
            ck(2 + p * g, p).start()
        cv(p * g, p).start()

    cq(0, NG - 1, 2, g - 2).start()
    ck(0, NG - 1, 2, g - 2).start()
    cq(0, NG - 1, 2, g - 2).wait()
    ck(0, NG - 1, 2, g - 2).wait()
    set_a(0)
    qk(R - 2, 0)
    for p in range(1, NG):
        set_a(p)
    qk(R - 1, 1)
    hs = 2 + (NG - 1) * g
    cq(hs, NG - 1).start()
    ck(hs, NG - 1).start()
    pr = sm(0)

    nit = (NH - 2) // G

    def body(it, carry):
        u0 = it * G
        st = ((p_scr[...], r_scr[...]), None)
        for j in range(G):
            st = step(u0, j, st, last=(j == G - 1))
        p_scr[...] = st[0][0]
        r_scr[...] = st[0][1]
        return carry

    p_scr[...] = pr[0]
    r_scr[...] = pr[1]
    lax.fori_loop(0, nit, body, 0)
    st = ((p_scr[...], r_scr[...]), None)
    u0 = nit * G
    for j in range(NH - u0):
        u = u0 + j
        st = step(u0, j, st, do_qk=(u + 2 < NH), do_sm=(u + 1 < NH), last=(u == NH - 1))
    for p in range(NG):
        last = max(u for u in range(0, NH, g) if (u % R) // g == p)
        co(last, p).wait()


@jax.jit
def pallas_standalone__mha_softmax__near_ridge_kernel(
    q: jax.Array,
    k: jax.Array,
    v: jax.Array,
):
    B, H, Sq, D = q.shape
    Sk = k.shape[2]
    c = (D ** -0.5) * _LOG2E
    NH = B * H
    R, g = _R, _g
    qT = jnp.swapaxes(q, -1, -2).reshape(NH, D, Sq)
    kT = jnp.swapaxes(k, -1, -2).reshape(NH, D, Sk)
    vT = jnp.swapaxes(v, -1, -2).reshape(NH, D, Sk)
    oT = pl.pallas_call(
        functools.partial(_mha_kernel, c=c, NH=NH),
        grid=(1,),
        in_specs=[pl.BlockSpec(memory_space=pl.ANY)] * 3,
        out_specs=pl.BlockSpec(memory_space=pl.ANY),
        out_shape=jax.ShapeDtypeStruct((NH, D, Sq), q.dtype),
        scratch_shapes=[
            pltpu.VMEM((R + 1, D, Sq), q.dtype), pltpu.VMEM((R, D, Sk), q.dtype),
            pltpu.VMEM((R, D, Sk), q.dtype), pltpu.VMEM((R + 1, D, Sq), q.dtype),
            pltpu.VMEM((2, Sq, Sk), jnp.float32),
            pltpu.VMEM((Sq, Sk), jnp.bfloat16), pltpu.VMEM((1, Sq), jnp.float32),
            pltpu.SemaphoreType.DMA((R // g,)), pltpu.SemaphoreType.DMA((R // g,)),
            pltpu.SemaphoreType.DMA((R // g,)), pltpu.SemaphoreType.DMA((R // g,)),
        ],
        compiler_params=pltpu.CompilerParams(
            vmem_limit_bytes=64 * 1024 * 1024,
            flags={"XLA_TPU_RESCHEDULE_DMA_DONES": True},
            disable_bounds_checks=True,
        ),
    )(qT, kT, vT)
    return jnp.swapaxes(oT.reshape(B, H, D, Sq), -1, -2)
```

```python
import functools

import jax
import jax.numpy as jnp
from jax import lax
import jax.experimental.pallas as pl
import jax.experimental.pallas.tpu as pltpu

_LOG2E = 1.4426950408889634
_G = 18
_R = 6
_g = 2
_NS = 3
_LEAD = 3
_QOFF = 4


def _mha_kernel(q_hbm, k_hbm, v_hbm, o_hbm,
                qb, kb, vb, ob, s_scr, p_scr, r_scr,
                sq, sk, sv, so, sp, *, c, NH):
    G, R, g, NS, LEAD, QOFF = _G, _R, _g, _NS, _LEAD, _QOFF
    NG = R // g
    ob[R, 0:16, 0:128] = jnp.zeros((16, 128), ob.dtype)
    zero = pl.program_id(0) // 4096

    def cq(h, p):
        return pltpu.make_async_copy(q_hbm.at[pl.ds(h, g)], qb.at[pl.ds(p * g, g)], sq.at[p])

    def ck(h, p):
        return pltpu.make_async_copy(k_hbm.at[pl.ds(h, g)], kb.at[pl.ds(p * g, g)], sk.at[p])

    def cv(h, p):
        return pltpu.make_async_copy(v_hbm.at[pl.ds(h, g)], vb.at[pl.ds(p * g, g)], sv.at[p])

    def co(h, p):
        return pltpu.make_async_copy(ob.at[pl.ds(p * g, g)], o_hbm.at[pl.ds(h, g)], so.at[p])

    def when(cond, fn):
        if isinstance(cond, bool):
            if cond:
                fn()
        else:
            pl.when(cond)(fn)

    def qk(slot, ss):
        s_scr[ss] = lax.dot_general(qb[slot], kb[slot], (((0,), (0,)), ((), ())),
                                    preferred_element_type=jnp.float32)

    def softmax(ss, dst=None):
        s = s_scr[ss]
        m = jnp.max(s, axis=1, keepdims=True)
        pb = jnp.exp2((s - m) * c).astype(jnp.bfloat16)
        l = jnp.sum(pb.astype(jnp.float32), axis=1, keepdims=True).T
        r0 = pl.reciprocal(l, approx=True)
        r = r0 + r0 * (1.0 - l * r0)
        if dst is not None:
            p_scr[dst] = pb
            r_scr[dst] = r
            return None
        return pb, r

    def do_qk(u, j, ws):
        hd = u + LEAD
        qs = (j + LEAD - QOFF) % R
        p = qs // g
        if qs % g == 0:
            cq(hd, p).wait()
            ck(hd, p).wait()
        qk(qs, ws)
        if qs % g == g - 1:
            hs = hd + 1 - g + R

            def refill():
                cq(hs, p).start()
                ck(hs, p).start()
            when(hs + g <= NH, refill)

    def do_pv(u, j, pr):
        slot = j % R
        if slot % g == 0:
            cv(u, slot // g).wait()
        pb, r = pr
        oT = lax.dot_general(vb[slot], pb, (((1,), (1,)), ((), ())),
                             preferred_element_type=jnp.float32)
        if slot % g == g - 1:
            hs = u + 1 - g + R
            when(hs + g <= NH, lambda: cv(hs, slot // g).start())
        return oT, r

    def finish(u, j, pend):
        slot = j % R
        p = slot // g
        if slot % g == 0:
            when(u >= R, lambda: co(u - R, p).wait())
        oT, r = pend
        ob[slot] = (oT * r).astype(ob.dtype)
        qb[R + zero, 0:16, 0:128] = ob[R + zero, 0:16, 0:128]
        if slot % g == g - 1:
            co(u + 1 - g, p).start()

    def step(u0, j, P, dst=None):
        u = u0 + j
        static = isinstance(u, int)
        pend = do_pv(u, j, P[0])
        if (not static) or u + 3 < NH:
            do_qk(u, j, (j + 3) % NS)
        finish(u, j, pend)
        pn = None
        if (not static) or u + 2 < NH:
            pn = softmax((j + 2) % NS, dst)
        return [P[1], pn]

    def one(hd):
        sl = (hd - QOFF) % R
        return (pltpu.make_async_copy(q_hbm.at[pl.ds(hd, 1)], qb.at[pl.ds(sl, 1)], sp.at[2 * hd]),
                pltpu.make_async_copy(k_hbm.at[pl.ds(hd, 1)], kb.at[pl.ds(sl, 1)], sp.at[2 * hd + 1]))

    A = [one(hd) for hd in range(QOFF)]

    def start_a(i):
        A[i][0].start()
        A[i][1].start()

    def wait_a(i):
        A[i][0].wait()
        A[i][1].wait()

    def start_qk_group(p):
        cq(QOFF + p * g, p).start()
        ck(QOFF + p * g, p).start()

    s0 = (0 - QOFF) % R
    start_a(0)
    start_a(1)
    wait_a(0)
    start_a(2)
    qk(s0, 0)
    wait_a(1)
    start_a(3)
    qk(s0 + 1, 1)
    wait_a(2)
    cv(0, 0).start()
    start_qk_group(0)
    qk(s0 + 2, 2)
    softmax(0, 0)
    wait_a(3)
    for p in range(1, NG - 1):
        start_qk_group(p)
    for p in range(1, NG):
        cv(p * g, p).start()
    softmax(1, 1)

    def carried():
        return [(p_scr[0], r_scr[0]), (p_scr[1], r_scr[1])]

    nit = (NH - LEAD) // G

    def body(it, carry):
        u0 = it * G
        P = carried()
        for j in range(G):
            P = step(u0, j, P, dst=(j - (G - 2) if j >= G - 2 else None))
        return carry

    lax.fori_loop(0, nit, body, 0)

    P = carried()
    u0 = nit * G
    for j in range(NH - u0):
        P = step(u0, j, P)
    for p in range(NG):
        last = max(u for u in range(0, NH, g) if (u % R) // g == p)
        co(last, p).wait()


@jax.jit
def pallas_standalone__mha_softmax__near_ridge_kernel(
    q: jax.Array,
    k: jax.Array,
    v: jax.Array,
):
    B, H, Sq, D = q.shape
    Sk = k.shape[2]
    c = (D ** -0.5) * _LOG2E
    NH = B * H
    R, g = _R, _g
    qT = jnp.swapaxes(q, -1, -2).reshape(NH, D, Sq)
    kT = jnp.swapaxes(k, -1, -2).reshape(NH, D, Sk)
    vT = jnp.swapaxes(v, -1, -2).reshape(NH, D, Sk)
    oT = pl.pallas_call(
        functools.partial(_mha_kernel, c=c, NH=NH),
        grid=(1,),
        in_specs=[pl.BlockSpec(memory_space=pl.ANY)] * 3,
        out_specs=pl.BlockSpec(memory_space=pl.ANY),
        out_shape=jax.ShapeDtypeStruct((NH, D, Sq), q.dtype),
        scratch_shapes=[
            pltpu.VMEM((R + 1, D, Sq), q.dtype),
            pltpu.VMEM((R, D, Sk), k.dtype),
            pltpu.VMEM((R, D, Sk), v.dtype),
            pltpu.VMEM((R + 1, D, Sq), q.dtype),
            pltpu.VMEM((_NS, Sq, Sk), jnp.float32),
            pltpu.VMEM((2, Sq, Sk), jnp.bfloat16),
            pltpu.VMEM((2, 1, Sq), jnp.float32),
            pltpu.SemaphoreType.DMA((R // g,)),
            pltpu.SemaphoreType.DMA((R // g,)),
            pltpu.SemaphoreType.DMA((R // g,)),
            pltpu.SemaphoreType.DMA((R // g,)),
            pltpu.SemaphoreType.DMA((2 * _QOFF,)),
        ],
        compiler_params=pltpu.CompilerParams(
            vmem_limit_bytes=64 * 1024 * 1024,
            flags={"XLA_TPU_RESCHEDULE_DMA_DONES": True},
            disable_bounds_checks=True,
        ),
    )(qT, kT, vT)
    return jnp.swapaxes(oT.reshape(B, H, D, Sq), -1, -2)
```

```python
import functools

import jax
import jax.numpy as jnp
from jax import lax
import jax.experimental.pallas as pl
import jax.experimental.pallas.tpu as pltpu

_LOG2E = 1.4426950408889634
_G = 36
_R = 6
_g = 2
_NS = 3
_LEAD = 3
_QOFF = 4


def _mha_kernel(q_hbm, k_hbm, v_hbm, o_hbm,
                qb, kb, vb, ob, s_scr, p_scr, r_scr,
                sq, sk, sv, so, sp, *, c, NH):
    G, R, g, NS, LEAD, QOFF = _G, _R, _g, _NS, _LEAD, _QOFF
    NG = R // g
    zero = pl.program_id(0) // 4096

    def cq(h, p):
        return pltpu.make_async_copy(q_hbm.at[pl.ds(h, g)], qb.at[pl.ds(p * g, g)], sq.at[p])

    def ck(h, p):
        return pltpu.make_async_copy(k_hbm.at[pl.ds(h, g)], kb.at[pl.ds(p * g, g)], sk.at[p])

    def cv(h, p):
        return pltpu.make_async_copy(v_hbm.at[pl.ds(h, g)], vb.at[pl.ds(p * g, g)], sv.at[p])

    def co(h, p):
        return pltpu.make_async_copy(ob.at[pl.ds(p * g, g)], o_hbm.at[pl.ds(h, g)], so.at[p])

    def co1(h, slot, p):
        return pltpu.make_async_copy(ob.at[pl.ds(slot, 1)], o_hbm.at[pl.ds(h, 1)], so.at[p])

    def when(cond, fn):
        if isinstance(cond, bool):
            if cond:
                fn()
        else:
            pl.when(cond)(fn)

    def qk(slot, ss):
        s_scr[ss] = lax.dot_general(qb[slot], kb[slot], (((0,), (0,)), ((), ())),
                                    preferred_element_type=jnp.float32)

    def softmax(ss, dst=None):
        s = s_scr[ss]
        m = jnp.max(s, axis=1, keepdims=True)
        pb = jnp.exp2((s - m) * c).astype(jnp.bfloat16)
        l = jnp.sum(pb.astype(jnp.float32), axis=1, keepdims=True).T
        r0 = pl.reciprocal(l, approx=True)
        r = r0 + r0 * (1.0 - l * r0)
        vb[R + zero, 0:1, 0:r.shape[1]] = r.astype(vb.dtype)
        if dst is not None:
            p_scr[dst] = pb
            r_scr[dst] = r
            return None
        return pb, r

    def step(u0, j, P, dst=None, tail=False):
        u = u0 + j
        static = isinstance(u, int)
        slot = j % R
        p = slot // g
        if slot % g == 0:
            cv(u, p).wait()
        oT = lax.dot_general(vb[slot], P[0][0], (((1,), (1,)), ((), ())),
                             preferred_element_type=jnp.float32)
        if slot % g == g - 1:
            hv = u + 1 - g + R
            when(hv + g <= NH, lambda: cv(hv, p).start())
        if (not static) or u + LEAD < NH:
            hd = u + LEAD
            qs = (j + LEAD - QOFF) % R
            pq = qs // g
            if qs % g == 0:
                cq(hd, pq).wait()
                ck(hd, pq).wait()
            qk(qs, (j + LEAD) % NS)
            if qs % g == g - 1:
                hq = hd + 1 - g + R

                def refill():
                    cq(hq, pq).start()
                    ck(hq, pq).start()
                when(hq + g <= NH, refill)
        if slot % g == 0:
            when(u >= R, lambda: co(u - R, p).wait())
        ob[slot] = (oT * P[0][1]).astype(ob.dtype)
        if tail and u >= NH - g:
            co1(u, slot, p).start()
        elif slot % g == g - 1:
            co(u + 1 - g, p).start()
        pn = None
        if (not static) or u + 2 < NH:
            pn = softmax((j + 2) % NS, dst)
        return [P[1], pn]

    def one(hd):
        sl = (hd - QOFF) % R
        return (pltpu.make_async_copy(q_hbm.at[pl.ds(hd, 1)], qb.at[pl.ds(sl, 1)], sp.at[2 * hd]),
                pltpu.make_async_copy(k_hbm.at[pl.ds(hd, 1)], kb.at[pl.ds(sl, 1)], sp.at[2 * hd + 1]))

    A = [one(hd) for hd in range(QOFF)]

    def start_a(i):
        A[i][0].start()
        A[i][1].start()

    def wait_a(i):
        A[i][0].wait()
        A[i][1].wait()

    def start_qk_group(p):
        cq(QOFF + p * g, p).start()
        ck(QOFF + p * g, p).start()

    s0 = (0 - QOFF) % R
    start_a(0)
    start_a(1)
    wait_a(0)
    start_a(2)
    qk(s0, 0)
    wait_a(1)
    start_a(3)
    qk(s0 + 1, 1)
    wait_a(2)
    cv(0, 0).start()
    start_qk_group(0)
    qk(s0 + 2, 2)
    softmax(0, 0)
    wait_a(3)
    for p in range(1, NG - 1):
        start_qk_group(p)
    for p in range(1, NG):
        cv(p * g, p).start()
    softmax(1, 1)

    def carried():
        return [(p_scr[0], r_scr[0]), (p_scr[1], r_scr[1])]

    nit = (NH - LEAD) // G

    def body(it, carry):
        u0 = it * G
        P = carried()
        for j in range(G):
            P = step(u0, j, P, dst=(j - (G - 2) if j >= G - 2 else None))
        return carry

    lax.fori_loop(0, nit, body, 0)

    P = carried()
    u0 = nit * G
    for j in range(NH - u0):
        P = step(u0, j, P, tail=True)
    for p in range(NG):
        last = max(u for u in range(0, NH, g) if (u % R) // g == p)
        if last == NH - g:
            for i in range(g):
                co1(last + i, (last % R) + i, p).wait()
        else:
            co(last, p).wait()


@jax.jit
def pallas_standalone__mha_softmax__near_ridge_kernel(
    q: jax.Array,
    k: jax.Array,
    v: jax.Array,
):
    B, H, Sq, D = q.shape
    Sk = k.shape[2]
    c = (D ** -0.5) * _LOG2E
    NH = B * H
    R, g = _R, _g
    qT = jnp.swapaxes(q, -1, -2).reshape(NH, D, Sq)
    kT = jnp.swapaxes(k, -1, -2).reshape(NH, D, Sk)
    vT = jnp.swapaxes(v, -1, -2).reshape(NH, D, Sk)
    oT = pl.pallas_call(
        functools.partial(_mha_kernel, c=c, NH=NH),
        grid=(1,),
        in_specs=[pl.BlockSpec(memory_space=pl.ANY)] * 3,
        out_specs=pl.BlockSpec(memory_space=pl.ANY),
        out_shape=jax.ShapeDtypeStruct((NH, D, Sq), q.dtype),
        scratch_shapes=[
            pltpu.VMEM((R, D, Sq), q.dtype),
            pltpu.VMEM((R, D, Sk), k.dtype),
            pltpu.VMEM((R + 1, D, Sk), v.dtype),
            pltpu.VMEM((R, D, Sq), q.dtype),
            pltpu.VMEM((_NS, Sq, Sk), jnp.float32),
            pltpu.VMEM((2, Sq, Sk), jnp.bfloat16),
            pltpu.VMEM((2, 1, Sq), jnp.float32),
            pltpu.SemaphoreType.DMA((R // g,)),
            pltpu.SemaphoreType.DMA((R // g,)),
            pltpu.SemaphoreType.DMA((R // g,)),
            pltpu.SemaphoreType.DMA((R // g,)),
            pltpu.SemaphoreType.DMA((2 * _QOFF,)),
        ],
        compiler_params=pltpu.CompilerParams(
            vmem_limit_bytes=32 * 1024 * 1024,
            flags={"XLA_TPU_RESCHEDULE_DMA_DONES": True},
        ),
    )(qT, kT, vT)
    return jnp.swapaxes(oT.reshape(B, H, D, Sq), -1, -2)
```
